```python
import jax
import jax.numpy as jnp

def _softmax(x, axis=-1):
    return jax.nn.softmax(x, axis=axis)

def _gelu(x):
    return jax.nn.gelu(x, approximate=True)

def _silu(x):
    return jax.nn.silu(x)

def _sigmoid(x):
    return jax.nn.sigmoid(x)

def _layernorm(x, axis=-1, eps=1e-05):
    m = jnp.mean(x, axis=axis, keepdims=True)
    v = jnp.var(x, axis=axis, keepdims=True)
    return (x - m) / jnp.sqrt(v + eps)

def _scatter_add(tgt, idx, src, axis=0):
    return tgt.at[idx].add(src)

def _segment_sum(src, seg, n):
    return jax.ops.segment_sum(src, seg, n)

class _Rng:

    def __init__(self, key):
        self._k = key

    def _next(self):
        self._k, sub = jax.random.split(self._k)
        return sub

    def normal(self, shape):
        return jax.random.normal(self._next(), shape, dtype=jnp.bfloat16)

    def randint(self, lo, hi, shape):
        return jax.random.randint(self._next(), shape, lo, hi, dtype=jnp.int32)

    def uniform(self, shape, lo=0.0, hi=1.0):
        return jax.random.uniform(self._next(), shape, jnp.bfloat16, lo, hi)

    def permutation(self, n):
        return jax.random.permutation(self._next(), n)
kernel_name = 'adaLN_cond__sliding_block_cached__mixer_s_mlp__decode'

def setup_inputs():
    _rng = _Rng(jax.random.key(int.from_bytes(__import__("os").urandom(4), "little")))
    _w = lambda a: (lambda t: t.astype(jnp.bfloat16) if jnp.issubdtype(t.dtype, jnp.floating) else t)(jnp.asarray(a))

    def _A_setup():
        B, Sq, D = (1, 1, 448)
        Hq, Hkv, Sk, Dh = (16, 8, 65536, 256)
        assert Hq % Hkv == 0, (Hq, Hkv)
        return {'x': _w((lambda *s: _rng.normal(s) * 0.05)(B, Sq, D)), 'k_cache': _w((lambda *s: _rng.normal(s) * 0.05)(B, Hkv, Sk, Dh)), 'v_cache': _w((lambda *s: _rng.normal(s) * 0.05)(B, Hkv, Sk, Dh)), 'wq': _w((lambda *s: _rng.normal(s) * 0.05)(D, Hq * Dh) * D ** (-0.5)), 'wo': _w((lambda *s: _rng.normal(s) * 0.05)(Hq * Dh, D) * (Hq * Dh) ** (-0.5))}
    _A_in = _A_setup()

    def _B_setup():
        B, S, D, F = (1, 1, 448, 1792)
        return {'x': _w((lambda *s: _rng.normal(s) * 0.05)(B, S, D)), 'w1': _w((lambda *s: _rng.normal(s) * 0.05)(D, D) * D ** (-0.5)), 'w2': _w((lambda *s: _rng.normal(s) * 0.05)(D, D) * D ** (-0.5)), 'w3': _w((lambda *s: _rng.normal(s) * 0.05)(D, F) * D ** (-0.5)), 'w4': _w((lambda *s: _rng.normal(s) * 0.05)(F, D) * F ** (-0.5))}
    _B_in = _B_setup()
    return {'A_x': _A_in['x'], 'A_k_cache': _A_in['k_cache'], 'A_v_cache': _A_in['v_cache'], 'A_wq': _A_in['wq'], 'A_wo': _A_in['wo'], 'B_x': _B_in['x'], 'B_w1': _B_in['w1'], 'B_w2': _B_in['w2'], 'B_w3': _B_in['w3'], 'B_w4': _B_in['w4'], 'c': _w((lambda *s: _rng.normal(s) * 0.05)(1, 448)), 'w_mod': _w((lambda *s: _rng.normal(s) * 0.05)(448, 6 * 448) * 448 ** (-0.5))}

def reference(A_x, A_k_cache, A_v_cache, A_wq, A_wo, B_x, B_w1, B_w2, B_w3, B_w4, c, w_mod):

    def _A_ref(x, k_cache, v_cache, wq, wo):
        B, Sq, D = x.shape
        Hq, Dh = (16, 256)
        Hkv, Sk = (k_cache.shape[1], k_cache.shape[2])
        W = min(4096, max(256, Sk // 4))
        rep = Hq // Hkv
        q = (lambda x, *d: x.transpose(*d))((x @ wq).reshape(B, Sq, Hq, Dh), 0, 2, 1, 3)
        k = jnp.repeat(k_cache[:, :, Sk - W:, :], rep, axis=1)
        v = jnp.repeat(v_cache[:, :, Sk - W:, :], rep, axis=1)
        scores = jnp.einsum('bhqd,bhkd->bhqk', q, k) * Dh ** (-0.5)
        p = _softmax(scores, axis=-1)
        o = jnp.einsum('bhqk,bhkd->bhqd', p, v)
        return (lambda x, *d: x.transpose(*d))(o, 0, 2, 1, 3).reshape(B, Sq, Hq * Dh) @ wo

    def _B_ref(x, w1, w2, w3, w4):
        B, S, D = x.shape
        h = _gelu(_layernorm(x, axis=-1) @ w1)
        c = D // 4
        g0 = jnp.pad(h[:, :, 0 * c:1 * c], ((0, 0), (1, 0), (0, 0)))[:, :S, :]
        g1 = jnp.pad(h[:, :, 1 * c:2 * c], ((0, 0), (0, 1), (0, 0)))[:, 1:, :]
        g2 = jnp.pad(h[:, :, 2 * c:3 * c], ((0, 0), (2, 0), (0, 0)))[:, :S, :]
        g3 = jnp.pad(h[:, :, 3 * c:], ((0, 0), (0, 2), (0, 0)))[:, 2:, :]
        hs = jnp.concatenate([g0, g1, g2, g3], axis=-1) @ w2
        x1 = x + hs
        h2 = _gelu(_layernorm(x1, axis=-1) @ w3) @ w4
        return x1 + h2
    x = A_x
    mod = (_silu(c) @ w_mod).reshape(c.shape[0], 6, 1, -1)
    sa, ca, ga, sb, cb, gb = (mod[:, 0].copy(), mod[:, 1].copy(), mod[:, 2].copy(), mod[:, 3].copy(), mod[:, 4].copy(), mod[:, 5].copy())
    h = _layernorm(x, axis=-1) * (1 + ca) + sa
    x = x + ga * _A_ref(h, A_k_cache, A_v_cache, A_wq, A_wo)
    h = _layernorm(x, axis=-1) * (1 + cb) + sb
    x = x + gb * _B_ref(h, B_w1, B_w2, B_w3, B_w4)
    return x
```

```python
import jax
import jax.numpy as jnp
from jax import lax
from jax.experimental import pallas as pl
from jax.experimental.pallas import tpu as pltpu

D, F = 448, 1792
HQ, HKV, DH = 16, 8, 256
EPS = 1e-5
ROWS = 8
BLOCK = 1024
BF16, F32 = jnp.bfloat16, jnp.float32
GATE = 18
HEAD = 26
DELTA = 16
SPLIT = 56
W4_CUT = 12
W4_LATE = ((8, 12), (24, 28))
SKEW, MOVE, MIX1, MIX0, MIXV = 0, 0, 0, 0, 1
GATE_GROUPS = (12, 10, 4, 2)
PLAN = 0
LAG, REST = 54, 1.5
VERBOSE = 0
NOCOMPUTE = 0
S_X, S_C, S_WM, S_WQ, S_WO, S_W3, S_K, S_V, S_LATE, S_W4, S_GATE = 0, 1, 2, 3, 4, 5, 6, 14, 22, 24, 26


def _layernorm(x):
    d = x - jnp.sum(x, axis=-1, keepdims=True) * (1.0 / D)
    return d * lax.rsqrt(jnp.sum(d * d, axis=-1, keepdims=True) * (1.0 / D) + EPS)


def _dot(a, b):
    return lax.dot_general(a, b, (((1,), (0,)), ((), ())), preferred_element_type=F32)


def _dot_t(a, b):
    return lax.dot_general(a, b, (((1,), (1,)), ((), ())), preferred_element_type=F32)


def _merge(*lists):
    keyed = [((i + 0.5) / len(xs), j, x) for j, xs in enumerate(lists) for i, x in enumerate(xs)]
    return [x for _, _, x in sorted(keyed, key=lambda k: k[:2])]


def _pieces(width, keep, size, rows):
    pieces = {}
    for t in range(rows * width):
        row, col = divmod(t, width)
        if col < keep:
            runs = pieces.setdefault(t // size, [])
            if runs and runs[-1][0] == row:
                runs[-1] = (row, runs[-1][1], runs[-1][2] + 1)
            else:
                runs.append((row, col, 1))
    return list(pieces.values())


def _kernel(x_hbm, c_hbm, wm_hbm, wq_hbm, k_hbm, v_hbm, wo_hbm, w3_hbm, w4_hbm, out_hbm,
            x_ref, c_ref, wm_ref, gate_ref, wq_ref, k_ref, v_ref, wo_ref, w3_ref, w4_ref,
            q_ref, p_ref, sum_ref, o_ref, attn_ref, mod_ref, silu_ref, out_ref, sems):
    blocks = k_ref.shape[1]
    window = blocks * BLOCK

    def cache(hbm, ref, sem, h, start, split):
        def piece(j):
            rows = pl.ds((start + j) % 64 * 16, 16)
            return [pltpu.make_async_copy(hbm.at[h, pl.ds(hbm.shape[1] - blocks, blocks), rows],
                                          ref.at[h, :, rows], sems.at[S_LATE + h // 2 % 2 if j >= split else sem + h])]
        return [piece(j) for j in range(64)]

    def pair(hbm, ref, sem, h, split=64):
        return _merge(cache(hbm, ref, sem, h, 0, split), cache(hbm, ref, sem, h + 2, DELTA, split))

    def weight(hbm, ref, sem, size):
        def copy(row, col, n):
            at = (slice(None), pl.ds(row * 8, 8), pl.ds(col * 128, n * 128))
            return pltpu.make_async_copy(hbm.at[at], ref.at[at], sems.at[sem(row)])
        return [[copy(*run) for run in piece]
                for piece in _pieces(hbm.shape[2] // 128, ref.shape[2] // 128, size, hbm.shape[1] // 8)]

    keys = {h: pair(k_hbm, k_ref, S_K, h) for h in (0, 1, 4, 5)}
    values = {h: pair(v_hbm, v_ref, S_V, h, SPLIT if h == 5 else 64) for h in (0, 1, 4, 5)}
    wq = weight(wq_hbm, wq_ref, lambda r: S_WQ, 4)
    wo = weight(wo_hbm, wo_ref, lambda r: S_WO, 4)
    wm = weight(wm_hbm, wm_ref, lambda r: S_WM, 8)
    w3 = weight(w3_hbm, w3_ref, lambda r: S_W3, 8)
    w4 = weight(w4_hbm, w4_ref, lambda r: S_W4 + any(lo <= r < hi for lo, hi in W4_LATE), 8)
    group = [g for g, n in enumerate(GATE_GROUPS) for _ in range(n)]
    gate = [[pltpu.make_async_copy(wm_hbm.at[:, pl.ds(r * 8, 8), pl.ds(GATE * 128, 384)],
                                   gate_ref.at[:, pl.ds(r * 8, 8)], sems.at[S_GATE + group[r]])] for r in range(28)]
    small = [[pltpu.make_async_copy(c_hbm, c_ref, sems.at[S_C]), pltpu.make_async_copy(x_hbm, x_ref, sems.at[S_X])]]

    k, v = keys, values
    cut = len(w4) * W4_CUT // 28
    if PLAN == 0:
        early = _merge(wq, wm) + small + wo
    elif PLAN == 1:
        early = _merge(wq, wm, wo) + small
    elif PLAN == 2:
        early = _merge(_merge(wq, wo[56:] + wo[:56]), wm) + small
    second = early + k[5] + v[1] + v[5]
    first = k[0] + k[1] + k[4] + v[0] + v[4]
    total = len(first + second + w3 + w4)
    move = (total + 1) // 2 + SKEW - len(first) - len(w4) + cut
    if MOVE == 0:
        first += _merge(w3[:move], w4[cut:cut + MIX1]) + w4[cut + MIX1:] + gate
        second = second[:-MIXV] + _merge(second[-MIXV:], w3[move:move + MIX0]) + w3[move + MIX0:] + w4[:cut]
    else:
        first += _merge(second[-move:], w4[cut:cut + MIX1]) + w4[cut + MIX1:] + gate
        second = second[:-move]
        second = second[:-MIXV] + _merge(second[-MIXV:], w3[:MIX0]) + w3[MIX0:] + w4[:cut]

    def landed(ref, sem):
        pltpu.make_async_copy(ref, ref, sems.at[sem]).wait()

    even = (lax.broadcasted_iota(jnp.int32, (ROWS, DH), 0) & 1) == 0
    live = {}

    def condition():
        for copy in small[0]:
            copy.wait()
        landed(wm_ref, S_WM)
        c = jnp.broadcast_to(c_ref[...].astype(F32), (ROWS, D))
        c = (c * jax.nn.sigmoid(c)).astype(BF16)
        mod = _dot(c, wm_ref[...].reshape(D, GATE * 128))
        for g in range(5):
            mod_ref[g] = mod[:, g * D:(g + 1) * D]
        mod_ref[5, :, :64] = mod[:, 5 * D:]
        pick = lax.broadcasted_iota(jnp.int32, (D, D), 0) == lax.broadcasted_iota(jnp.int32, (D, D), 1)
        column = jnp.sum(jnp.where(pick, jnp.broadcast_to(c.astype(F32)[:1], (D, D)), 0.0), axis=1, keepdims=True)
        silu_ref[...] = jnp.broadcast_to(column, (D, 128))

    def queries():
        x = jnp.broadcast_to(x_ref[0].astype(F32), (ROWS, D))
        h_in = (_layernorm(x) * (1.0 + mod_ref[1]) + mod_ref[0]).astype(BF16)
        landed(wq_ref, S_WQ)
        for h in range(HKV):
            q = _dot(h_in, wq_ref[:, :, h * 2 * DH:(h + 1) * 2 * DH].reshape(D, 2 * DH)) * DH ** -0.5
            q_ref[h] = jnp.where(even, q[:, :DH], q[:, DH:])

    def scores(h):
        landed(k_ref.at[h], S_K + h)
        s = _dot_t(q_ref[h].astype(BF16), k_ref[h].reshape(window, DH))
        m = s[:, :128]
        for t in range(1, window // 128):
            m = jnp.maximum(m, s[:, t * 128:(t + 1) * 128])
        p = jnp.exp(s - jnp.max(m, axis=-1, keepdims=True))
        total = p[:, :128]
        for t in range(1, window // 128):
            total = total + p[:, t * 128:(t + 1) * 128]
        p_ref[h] = p
        sum_ref[h] = jnp.broadcast_to(1.0 / jnp.sum(total, axis=-1, keepdims=True), (ROWS, DH))

    def context(h, lo=0, hi=64):
        landed(v_ref.at[h, :, pl.ds(0, (hi - lo) * 16)], S_LATE + h // 2 % 2 if lo else S_V + h)
        tiles = [(b, (j + h // 2 % 2 * DELTA) % 64 * 16) for b in range(blocks) for j in range(lo, hi, 8)]
        p = jnp.concatenate([p_ref[h, :, b * BLOCK + r:b * BLOCK + r + 128] for b, r in tiles], axis=1)
        o = _dot(p.astype(BF16), jnp.concatenate([v_ref[h, b, r:r + 128] for b, r in tiles], axis=0))
        if lo:
            o = o + o_ref[h, :, :DH]
        if hi < 64:
            o_ref[h, :, :DH] = o
        else:
            o = o * sum_ref[h]
            o_ref[h] = jnp.concatenate([jnp.where(even, o, 0.0), jnp.where(even, 0.0, o)], axis=1)

    def project(h):
        start = "attn" not in live
        if start:
            landed(wo_ref, S_WO)
        y = _dot_t(o_ref[h].astype(BF16), wo_ref[:, :, h * 2 * DH:(h + 1) * 2 * DH].reshape(D, 2 * DH))
        attn_ref[...] = y if start else attn_ref[...] + y
        live["attn"] = True

    def normalize():
        attn = attn_ref[...]
        x = jnp.broadcast_to(x_ref[0].astype(F32), (ROWS, D))
        x = x + mod_ref[2] * (attn + pltpu.roll(attn, 1, 0))
        h_mlp = _layernorm(x) * (1.0 + mod_ref[4]) + mod_ref[3]
        live["normed"] = _layernorm(h_mlp).astype(BF16)
        mod_ref[0] = x
        mod_ref[1] = h_mlp

    queue = []
    for j in range(max(len(first), len(second) + HEAD)):
        queue += [(1, copy) for copy in (first[j] if j < len(first) else ())]
        queue += [(0, copy) for copy in (second[j - HEAD] if HEAD <= j < len(second) + HEAD else ())]

    def ready(pieces):
        ids = {id(copy) for piece in pieces for copy in piece}
        slow = [j for j, (priority, _) in enumerate(queue) if priority]
        return LAG + max([slow[min(i + HEAD, len(slow) - 1)] for i, j in enumerate(slow) if id(queue[j][1]) in ids] +
                         [j for j, (_, copy) in enumerate(queue) if id(copy) in ids])

    steps = [(ready(wm + small), 8, condition), (ready(wq), 10, queries)]
    for h in sorted((0, 1, 4, 5), key=lambda h: ready(keys[h])):
        steps += [(ready(keys[h]), 12, lambda h=h + i: scores(h)) for i in (0, 2)]
    done = []
    for h in sorted((0, 1, 4, 5), key=lambda h: ready(values[h])):
        if h == 5 and SPLIT < 64:
            steps += [(ready(values[h][:2 * SPLIT]), 6, lambda h=h + i: context(h, 0, SPLIT)) for i in (0, 2)]
        steps += [(ready(values[h]), 0 if h == 5 else 8, lambda h=h + i: context(h, SPLIT % 64 if h in (5, 7) else 0)) for i in (0, 2)]
        done += [h, h + 2]
        if ready(wo) <= ready(values[h]) or len(steps) >= 18:
            steps += [(ready(wo), 3, lambda h=h: project(h)) for h in done]
            done = []
    steps += [(0, 0, normalize)]
    work, at = [], 0
    n = len(steps) - 5 - 2 * (SPLIT < 64)
    steps[n - 4:n + 2] = sorted(steps[n - 4:n + 2], key=lambda s: max(s[0], ready(values[4])) if s[1] != 6 else s[0])
    for slot, rest, step in steps:
        at = max(at, slot)
        work.append((at, step))
        at += rest * REST
    if VERBOSE:
        print(len(first), len(second), [w[0] for w in work])
    if NOCOMPUTE in (1, 3):
        work = []

    for j, (priority, copy) in enumerate(queue):
        copy.start(priority=priority)
        while work and work[0][0] <= j:
            work.pop(0)[1]()
    for _, step in work:
        step()

    store = pltpu.make_async_copy(out_ref, out_hbm, sems.at[S_X])
    if NOCOMPUTE in (1, 3):
        for copy in small[0]:
            copy.wait()
        for ref, sem in [(wm_ref, S_WM), (wq_ref, S_WQ), (wo_ref, S_WO)] + [(k_ref.at[h], S_K + h) for h in range(8)] + [(v_ref.at[h, :, pl.ds(0, 16 * (SPLIT if h in (5, 7) else 64))], S_V + h) for h in range(8)] + [(v_ref.at[0, :, pl.ds(0, 1024 - 16 * SPLIT)], S_LATE + i) for i in range(2 * (SPLIT < 64))]:
            landed(ref, sem)
        live["normed"] = mod_ref[0].astype(BF16)
    if NOCOMPUTE in (1, 2):
        landed(w3_ref, S_W3)
        late = sum(hi - lo for lo, hi in W4_LATE) * 8
        landed(w4_ref.at[:, pl.ds(0, 224 - late)], S_W4)
        landed(w4_ref.at[:, pl.ds(0, late)], S_W4 + 1)
        r0 = 0
        for g, n in enumerate(GATE_GROUPS):
            landed(gate_ref.at[:, pl.ds(r0, n * 8)], S_GATE + g)
            r0 += n * 8
        out_ref[...] = x_ref[...]
        store.start()
        store.wait()
        return

    landed(w3_ref, S_W3)
    hidden = jax.nn.gelu(_dot(live["normed"], w3_ref[...].reshape(D, F)), approximate=True).astype(BF16)
    half = D // 2
    edges = sorted({0, 28} | {e for span in W4_LATE for e in span})
    parts = {}
    for i in range(2):
        spans = [(s, lo * 8, hi * 8) for s in range(2) for lo, hi in zip(edges, edges[1:])
                 if any(a <= lo < b for a, b in W4_LATE) == i]
        rows = sum(hi - lo for _, lo, hi in spans)
        landed(w4_ref.at[:, pl.ds(0, rows // 2)], S_W4 + i)
        y = _dot_t(hidden, jnp.concatenate([w4_ref[s, lo:hi] for s, lo, hi in spans], axis=0))
        at = 0
        for span in spans:
            parts[span] = y[:, at:at + span[2] - span[1]]
            at += span[2] - span[1]
    y = mod_ref[1] + jnp.concatenate([parts[span] for span in sorted(parts)], axis=1)

    acc, r0 = None, 0
    for g, n in enumerate(GATE_GROUPS):
        landed(gate_ref.at[:, pl.ds(r0, n * 8)], S_GATE + g)
        for s in range(2):
            w = gate_ref[s, r0:r0 + n * 8].astype(F32)
            for r in range(0, n * 8, 8):
                t = w[r:r + 8] * jnp.concatenate([silu_ref[s * half + r0 + r:s * half + r0 + r + 8]] * 3, axis=1)
                acc = t if acc is None else acc + t
        r0 += n * 8
    gb = jnp.concatenate([mod_ref[5, :1, :64], jnp.sum(acc, axis=0, keepdims=True)], axis=1)
    out_ref[0] = (mod_ref[0, :1] + gb * y[:1]).astype(BF16)
    store.start()
    store.wait()


@jax.jit
def pallas_adaLN_cond__sliding_block_cached__mixer_s_mlp__decode_kernel(
    A_x, A_k_cache, A_v_cache, A_wq, A_wo, B_x, B_w1, B_w2, B_w3, B_w4, c, w_mod,
):
    keys = A_k_cache.shape[2]
    window = min(4096, max(256, keys // 4))
    assert A_x.shape == (1, 1, D) and A_k_cache.shape == (1, HKV, keys, DH) and window == 4096 and keys % BLOCK == 0
    hbm = pl.BlockSpec(memory_space=pltpu.HBM)
    blocked = (HKV, keys // BLOCK, BLOCK, DH)
    return pl.pallas_call(
        _kernel,
        out_shape=jax.ShapeDtypeStruct(A_x.shape, A_x.dtype),
        in_specs=[hbm] * 9,
        out_specs=hbm,
        scratch_shapes=[
            pltpu.VMEM((1, 1, D), BF16),
            pltpu.VMEM((1, D), BF16),
            pltpu.VMEM((2, D // 2, GATE * 128), BF16),
            pltpu.VMEM((2, D // 2, 384), BF16),
            pltpu.VMEM((4, D // 4, HQ * DH), BF16),
            pltpu.VMEM((HKV, window // BLOCK, BLOCK, DH), BF16),
            pltpu.VMEM((HKV, window // BLOCK, BLOCK, DH), BF16),
            pltpu.VMEM((4, D // 4, HQ * DH), BF16),
            pltpu.VMEM((2, D // 2, F), BF16),
            pltpu.VMEM((2, D // 2, F), BF16),
            pltpu.VMEM((HKV, ROWS, DH), F32),
            pltpu.VMEM((HKV, ROWS, window), F32),
            pltpu.VMEM((HKV, ROWS, DH), F32),
            pltpu.VMEM((HKV, ROWS, 2 * DH), F32),
            pltpu.VMEM((ROWS, D), F32),
            pltpu.VMEM((6, ROWS, D), F32),
            pltpu.VMEM((D, 128), F32),
            pltpu.VMEM((1, 1, D), BF16),
            pltpu.SemaphoreType.DMA((S_GATE + len(GATE_GROUPS),)),
        ],
        compiler_params=pltpu.CompilerParams(
            vmem_limit_bytes=100 * 2**20,
            disable_semaphore_checks=True,
        ),
        name="adaln_decode",
    )(A_x, c, w_mod.reshape(2, D // 2, 6 * D), A_wq.reshape(4, D // 4, HQ * DH), A_k_cache.reshape(blocked),
      A_v_cache.reshape(blocked), A_wo.T.reshape(4, D // 4, HQ * DH), B_w3.reshape(2, D // 2, F),
      B_w4.T.reshape(2, D // 2, F))
```

```python
import functools

import jax
import jax.numpy as jnp
from jax import lax
from jax.experimental import pallas as pl
from jax.experimental.pallas import tpu as pltpu

D, F = 448, 1792
HQ, HKV, DH = 16, 8, 256
EPS = 1e-5
BF16, F32 = jnp.bfloat16, jnp.float32
ROWS = 8

HALF = D // 2
TILE_ROWS = HALF // 8
BLOCK, SEGMENT = 1024, 16
PIECES = BLOCK // SEGMENT
PAIRS = (0, 1, 4, 5)
STAGGER = 16
LAST, LAST_EARLY = 5, 56
GATE = 18
GATE_GROUPS = (12, 10, 4, 2)
W4_BLOCKS = (((6, 14), (14, 22)), ((0, 4), (24, 28)), ((4, 6), (22, 24)))
BACKLOG = 25
IN_FLIGHT = 54

S_X, S_C, S_WM, S_WQ, S_WO, S_W3, S_K, S_V, S_REST, S_W4 = 0, 1, 2, 3, 4, 5, 6, 14, 22, 24
S_GATE = S_W4 + 2 * len(W4_BLOCKS)


def _layernorm(x):
    d = x - jnp.sum(x, axis=-1, keepdims=True) * (1.0 / D)
    return d * lax.rsqrt(jnp.sum(d * d, axis=-1, keepdims=True) * (1.0 / D) + EPS)


def _dot(a, b):
    return lax.dot_general(a, b, (((1,), (0,)), ((), ())), preferred_element_type=F32)


def _dot_t(a, b):
    return lax.dot_general(a, b, (((1,), (1,)), ((), ())), preferred_element_type=F32)


def _fold(op, x):
    return functools.reduce(op, [x[:, t:t + 128] for t in range(0, x.shape[1], 128)])


def _merge(*lists):
    keyed = [((i + 0.5) / len(xs), j, x) for j, xs in enumerate(lists) for i, x in enumerate(xs)]
    return [x for _, _, x in sorted(keyed, key=lambda k: k[:2])]


def _both_ends(xs):
    return _merge(xs[:len(xs) // 2], xs[len(xs) // 2:])


def _cut(width, columns, lo, hi):
    pieces = {}
    for t in range(lo * width, hi * width):
        row, col = divmod(t, width)
        if col < columns:
            runs = pieces.setdefault(t // 8, [])
            if runs and runs[-1][0] == row:
                runs[-1] = (row, runs[-1][1], runs[-1][2] + 1)
            else:
                runs.append((row, col, 1))
    return list(pieces.values())


def _kernel(x_hbm, c_hbm, wm_hbm, wq_hbm, k_hbm, v_hbm, wo_hbm, w3_hbm, w4_hbm, out_hbm,
            x_ref, c_ref, wm_ref, gate_ref, wq_ref, k_ref, v_ref, wo_ref, w3_ref, w4_ref,
            q_ref, p_ref, scale_ref, o_ref, attn_ref, mod_ref, silu_ref, out_ref, sems):
    blocks = k_ref.shape[2]
    keys_per_piece = blocks * SEGMENT

    def cache(hbm, ref, h, sem):
        def piece(head, j):
            rows = pl.ds((j + (head - h) // 2 * STAGGER) % PIECES * SEGMENT, SEGMENT)
            return [pltpu.make_async_copy(hbm.at[head, pl.ds(hbm.shape[1] - blocks, blocks), rows],
                                          ref.at[head, j], sems.at[sem(head, j)])]
        return [piece(head, j) for j in range(PIECES) for head in (h, h + 2)]

    def value_sem(head, j):
        return S_REST + (head - LAST) // 2 if head in (LAST, LAST + 2) and j >= LAST_EARLY else S_V + head

    def weight(hbm, ref, sem, lo=0, hi=TILE_ROWS):
        def copy(row, col, n):
            at = (slice(None), pl.ds(row * 8, 8), pl.ds(col * 128, n * 128))
            return pltpu.make_async_copy(hbm.at[at], ref.at[at], sems.at[sem])
        return [[copy(*run) for run in piece] for piece in _cut(hbm.shape[2] // 128, ref.shape[2] // 128, lo, hi)]

    k = {h: cache(k_hbm, k_ref, h, lambda head, j: S_K + head) for h in PAIRS}
    v = {h: cache(v_hbm, v_ref, h, value_sem) for h in PAIRS}
    wm, wq, wo, w3 = (weight(*args) for args in (
        (wm_hbm, wm_ref, S_WM), (wq_hbm, wq_ref, S_WQ), (wo_hbm, wo_ref, S_WO), (w3_hbm, w3_ref, S_W3)))
    w4 = [[piece for i, spans in enumerate(W4_BLOCKS) for piece in weight(w4_hbm, w4_ref, S_W4 + 2 * i + q, *spans[q])]
          for q in range(2)]
    gate = [[pltpu.make_async_copy(wm_hbm.at[:, pl.ds(row * 8, 8), pl.ds(GATE * 128, gate_ref.shape[2])],
                                   gate_ref.at[:, pl.ds(row * 8, 8)], sems.at[S_GATE + g])]
            for row, g in enumerate(g for g, n in enumerate(GATE_GROUPS) for _ in range(n))]
    inputs = [pltpu.make_async_copy(c_hbm, c_ref, sems.at[S_C]), pltpu.make_async_copy(x_hbm, x_ref, sems.at[S_X])]

    first = (k[0] + k[1] + _merge(k[4], _both_ends(wo)[-16:]) + v[0] + v[4]
             + _merge(w3[:30], w4[1][:6]) + w4[1][6:] + gate)
    second = (_merge(_both_ends(wq), wm) + [inputs] + _both_ends(wo)[:-16] + k[5] + v[1] + v[5][:-24]
              + _merge(v[5][-24:], w3[30:38]) + _merge(w3[38:], w4[0][:4]) + w4[0][4:])
    queue = []
    for j in range(max(len(first), len(second) + BACKLOG)):
        queue += [(1, copy) for piece in first[j:j + 1] for copy in piece]
        queue += [(0, copy) for piece in second[max(j - BACKLOG, 0):max(j + 1 - BACKLOG, 0)] for copy in piece]

    def ready(pieces):
        wanted = {id(copy) for piece in pieces for copy in piece}
        slow = [j for j, (priority, _) in enumerate(queue) if priority]
        return IN_FLIGHT + max(
            [j for j, (_, copy) in enumerate(queue) if id(copy) in wanted]
            + [slow[min(i + BACKLOG, len(slow) - 1)] for i, j in enumerate(slow) if id(queue[j][1]) in wanted])

    def landed(ref, sem):
        pltpu.make_async_copy(ref, ref, sems.at[sem]).wait()

    even = (lax.broadcasted_iota(jnp.int32, (ROWS, DH), 0) & 1) == 0
    head_columns = lambda ref, h: ref[:, :, h * 2 * DH:(h + 1) * 2 * DH].reshape(D, 2 * DH)
    residual = lambda: jnp.broadcast_to(x_ref[0].astype(F32), (ROWS, D))

    def condition():
        for copy in inputs:
            copy.wait()
        landed(wm_ref, S_WM)
        c = jnp.broadcast_to(c_ref[...].astype(F32), (ROWS, D))
        c = (c * jax.nn.sigmoid(c)).astype(BF16)
        mod = _dot(c, wm_ref[...].reshape(D, GATE * 128))
        for g in range(5):
            mod_ref[g] = mod[:, g * D:(g + 1) * D]
        mod_ref[5, :, :GATE * 128 - 5 * D] = mod[:, 5 * D:]
        diagonal = lax.broadcasted_iota(jnp.int32, (D, D), 0) == lax.broadcasted_iota(jnp.int32, (D, D), 1)
        column = jnp.sum(jnp.where(diagonal, jnp.broadcast_to(c.astype(F32)[:1], (D, D)), 0.0), axis=1, keepdims=True)
        silu_ref[...] = jnp.broadcast_to(column, (D, 128))
        attn_ref[...] = jnp.zeros((ROWS, D), F32)

    def queries():
        h_in = (_layernorm(residual()) * (1.0 + mod_ref[1]) + mod_ref[0]).astype(BF16)
        landed(wq_ref, S_WQ)
        for h in range(HKV):
            q = _dot(h_in, head_columns(wq_ref, h)) * DH ** -0.5
            q_ref[h] = jnp.where(even, q[:, :DH], q[:, DH:])

    def weights(h):
        landed(k_ref.at[h], S_K + h)
        s = _dot_t(q_ref[h].astype(BF16), k_ref[h].reshape(PIECES * keys_per_piece, DH))
        p = jnp.exp(s - jnp.max(_fold(jnp.maximum, s), axis=-1, keepdims=True))
        p_ref[h] = p
        scale_ref[h] = jnp.broadcast_to(1.0 / jnp.sum(_fold(jnp.add, p), axis=-1, keepdims=True), (ROWS, DH))

    def context(h, lo, hi):
        landed(v_ref.at[h, pl.ds(lo, hi - lo)], value_sem(h, lo))
        o = _dot(p_ref[h, :, lo * keys_per_piece:hi * keys_per_piece].astype(BF16),
                 v_ref[h, lo:hi].reshape((hi - lo) * keys_per_piece, DH))
        if lo > 0:
            o = o + o_ref[h]
        o_ref[h] = o * scale_ref[h] if hi == PIECES else o

    def project(h):
        o = o_ref[h]
        o = jnp.concatenate([jnp.where(even, o, 0.0), jnp.where(even, 0.0, o)], axis=1)
        attn_ref[...] += _dot_t(o.astype(BF16), head_columns(wo_ref, h))

    def normalize():
        attn = attn_ref[...]
        x = residual() + mod_ref[2] * (attn + pltpu.roll(attn, 1, 0))
        h_mlp = _layernorm(x) * (1.0 + mod_ref[4]) + mod_ref[3]
        mod_ref[0], mod_ref[1], mod_ref[2] = x, h_mlp, _layernorm(h_mlp)

    steps = [(ready(wm + [inputs]), 12, condition), (ready(wq), 15, queries)]
    for h in PAIRS:
        steps += [(ready(k[h]), 18, functools.partial(weights, head)) for head in (h, h + 2)]
    steps += [(ready(wo), 0, functools.partial(landed, wo_ref, S_WO))]
    for h in PAIRS:
        for lo, hi in ((0, LAST_EARLY), (LAST_EARLY, PIECES)) if h == LAST else ((0, PIECES),):
            steps += [(ready(v[h][:2 * hi]), (hi - lo) // 6, functools.partial(context, head, lo, hi))
                      for head in (h, h + 2)]
        steps += [(0, 4, functools.partial(project, head)) for head in (h, h + 2)]
    steps += [(0, 0, normalize)]

    earliest = 0
    for j, (priority, copy) in enumerate(queue):
        copy.start(priority=priority)
        while steps and j >= max(earliest, steps[0][0]):
            _, rest, step = steps.pop(0)
            step()
            earliest = j + rest
    for _, _, step in steps:
        step()

    landed(w3_ref, S_W3)
    hidden = jax.nn.gelu(_dot(mod_ref[2].astype(BF16), w3_ref[...].reshape(D, F)), approximate=True).astype(BF16)

    group = lax.broadcasted_iota(jnp.int32, (ROWS, 128), 1) // 16
    y = [jnp.zeros((ROWS, 128), F32)] * 4
    for i, spans in enumerate(W4_BLOCKS):
        for q, (lo, hi) in enumerate(spans):
            landed(w4_ref.at[:, pl.ds(lo * 8, (hi - lo) * 8)], S_W4 + 2 * i + q)
        channels = [s * HALF + r for s in range(2) for lo, hi in spans for r in range(lo * 8, hi * 8, 16)]
        while channels:
            lanes = {}
            for ch in channels:
                lanes.setdefault(ch % 128 // 16, ch)
            chosen = [lanes[g] for g in range(len(lanes))]
            channels = [ch for ch in channels if ch not in chosen]
            product = _dot_t(hidden, jnp.concatenate(
                [w4_ref[ch // HALF, pl.ds(ch % HALF, 16)] for ch in chosen], axis=0))
            if len(chosen) < 8:
                product = jnp.concatenate([product, jnp.zeros((ROWS, 128 - 16 * len(chosen)), F32)], axis=1)
            for g, ch in enumerate(chosen):
                y[ch // 128] = jnp.where(group == g, product, y[ch // 128])
    y = mod_ref[1] + jnp.concatenate(y, axis=1)[:, :D]

    total, lo = None, 0
    for g, n in enumerate(GATE_GROUPS):
        landed(gate_ref.at[:, pl.ds(lo, n * 8)], S_GATE + g)
        for s in range(2):
            w = gate_ref[s, lo:lo + n * 8].astype(F32)
            for r in range(0, n * 8, 8):
                term = w[r:r + 8] * jnp.concatenate([silu_ref[pl.ds(s * HALF + lo + r, 8)]] * 3, axis=1)
                total = term if total is None else total + term
        lo += n * 8
    gb = jnp.concatenate([mod_ref[5, :1, :GATE * 128 - 5 * D], jnp.sum(total, axis=0, keepdims=True)], axis=1)
    out_ref[0] = (mod_ref[0, :1] + gb * y[:1]).astype(BF16)
    store = pltpu.make_async_copy(out_ref, out_hbm, sems.at[S_X])
    store.start()
    store.wait()


@jax.jit
def pallas_adaLN_cond__sliding_block_cached__mixer_s_mlp__decode_kernel(
    A_x: jax.Array,
    A_k_cache: jax.Array,
    A_v_cache: jax.Array,
    A_wq: jax.Array,
    A_wo: jax.Array,
    B_x: jax.Array,
    B_w1: jax.Array,
    B_w2: jax.Array,
    B_w3: jax.Array,
    B_w4: jax.Array,
    c: jax.Array,
    w_mod: jax.Array,
):
    keys = A_k_cache.shape[2]
    window = min(4096, max(256, keys // 4))
    assert A_x.shape == (1, 1, D) and A_k_cache.shape == (1, HKV, keys, DH)
    assert window % BLOCK == 0 and keys % BLOCK == 0
    hbm = pl.BlockSpec(memory_space=pltpu.HBM)
    blocked = lambda cache: cache.reshape(HKV, keys // BLOCK, BLOCK, DH)
    halved = lambda w: w.reshape(2, HALF, w.shape[1])
    landing_order = (HKV, PIECES, window // BLOCK, SEGMENT, DH)
    return pl.pallas_call(
        _kernel,
        out_shape=jax.ShapeDtypeStruct(A_x.shape, A_x.dtype),
        in_specs=[hbm] * 9,
        out_specs=hbm,
        scratch_shapes=[
            pltpu.VMEM((1, 1, D), BF16),
            pltpu.VMEM((1, D), BF16),
            pltpu.VMEM((2, HALF, GATE * 128), BF16),
            pltpu.VMEM((2, HALF, 6 * D - GATE * 128), BF16),
            pltpu.VMEM((2, HALF, HQ * DH), BF16),
            pltpu.VMEM(landing_order, BF16),
            pltpu.VMEM(landing_order, BF16),
            pltpu.VMEM((2, HALF, HQ * DH), BF16),
            pltpu.VMEM((2, HALF, F), BF16),
            pltpu.VMEM((2, HALF, F), BF16),
            pltpu.VMEM((HKV, ROWS, DH), F32),
            pltpu.VMEM((HKV, ROWS, window), F32),
            pltpu.VMEM((HKV, ROWS, DH), F32),
            pltpu.VMEM((HKV, ROWS, DH), F32),
            pltpu.VMEM((ROWS, D), F32),
            pltpu.VMEM((6, ROWS, D), F32),
            pltpu.VMEM((D, 128), F32),
            pltpu.VMEM((1, 1, D), BF16),
            pltpu.SemaphoreType.DMA((S_GATE + len(GATE_GROUPS),)),
        ],
        compiler_params=pltpu.CompilerParams(
            vmem_limit_bytes=100 * 2**20,
            disable_semaphore_checks=True,
        ),
        name="adaln_decode",
    )(A_x, c, halved(w_mod), halved(A_wq), blocked(A_k_cache), blocked(A_v_cache), halved(A_wo.T),
      halved(B_w3), halved(B_w4.T))
```

```python
import functools

import jax
import jax.numpy as jnp
from jax import lax
from jax.experimental import pallas as pl
from jax.experimental.pallas import tpu as pltpu

D, F = 448, 1792
HQ, HKV, DH = 16, 8, 256
EPS = 1e-5
BF16, F32 = jnp.bfloat16, jnp.float32
ROWS = 8

HALF = D // 2
TILE_ROWS = HALF // 8
BLOCK, SEGMENT = 1024, 16
PIECES = BLOCK // SEGMENT
PAIRS = (0, 1, 4, 5)
STAGGER = 16
LAST, LAST_EARLY = 5, 56
GATE = 18
GATE_GROUPS = (12, 10, 4, 2)
W4_BLOCKS = (((6, 14), (14, 22)), ((0, 4), (24, 28)), ((4, 6), (22, 24)))
BACKLOG = 26
IN_FLIGHT = 54

S_X, S_C, S_WM, S_WQ, S_WO, S_W3, S_K, S_V, S_REST, S_W4 = 0, 1, 2, 3, 4, 5, 6, 14, 22, 24
S_GATE = S_W4 + 2 * len(W4_BLOCKS)


def _layernorm(x):
    d = x - jnp.sum(x, axis=-1, keepdims=True) * (1.0 / D)
    return d * lax.rsqrt(jnp.sum(d * d, axis=-1, keepdims=True) * (1.0 / D) + EPS)


def _dot(a, b):
    return lax.dot_general(a, b, (((1,), (0,)), ((), ())), preferred_element_type=F32)


def _dot_t(a, b):
    return lax.dot_general(a, b, (((1,), (1,)), ((), ())), preferred_element_type=F32)


def _fold(op, x):
    return functools.reduce(op, [x[:, t:t + 128] for t in range(0, x.shape[1], 128)])


def _merge(*lists):
    keyed = [((i + 0.5) / len(xs), j, x) for j, xs in enumerate(lists) for i, x in enumerate(xs)]
    return [x for _, _, x in sorted(keyed, key=lambda k: k[:2])]


def _both_ends(xs):
    return _merge(xs[:len(xs) // 2], xs[len(xs) // 2:])


def _cut(width, columns, lo, hi):
    pieces = {}
    for t in range(lo * width, hi * width):
        row, col = divmod(t, width)
        if col < columns:
            runs = pieces.setdefault(t // 8, [])
            if runs and runs[-1][0] == row:
                runs[-1] = (row, runs[-1][1], runs[-1][2] + 1)
            else:
                runs.append((row, col, 1))
    return list(pieces.values())


def _kernel(x_hbm, c_hbm, wm_hbm, wq_hbm, k_hbm, v_hbm, wo_hbm, w3_hbm, w4_hbm, out_hbm,
            x_ref, c_ref, wm_ref, gate_ref, wq_ref, k_ref, v_ref, wo_ref, w3_ref, w4_ref,
            q_ref, p_ref, scale_ref, o_ref, attn_ref, mod_ref, silu_ref, out_ref, sems):
    blocks = k_ref.shape[2]
    keys_per_piece = blocks * SEGMENT

    def cache(hbm, ref, h, sem):
        def piece(head, j):
            rows = pl.ds(((j ^ 1) + (head - h) // 2 * STAGGER) % PIECES * SEGMENT, SEGMENT)
            return [pltpu.make_async_copy(hbm.at[head, pl.ds(hbm.shape[1] - blocks, blocks), rows],
                                          ref.at[head, j], sems.at[sem(head, j)])]
        return [piece(head, j) for j in range(PIECES) for head in (h, h + 2)]

    def value_sem(head, j):
        return S_REST + (head - LAST) // 2 if head in (LAST, LAST + 2) and j >= LAST_EARLY else S_V + head

    def weight(hbm, ref, sem, lo=0, hi=TILE_ROWS):
        def copy(row, col, n):
            at = (slice(None), pl.ds(row * 8, 8), pl.ds(col * 128, n * 128))
            return pltpu.make_async_copy(hbm.at[at], ref.at[at], sems.at[sem])
        return [[copy(*run) for run in piece] for piece in _cut(hbm.shape[2] // 128, ref.shape[2] // 128, lo, hi)]

    k = {h: cache(k_hbm, k_ref, h, lambda head, j: S_K + head) for h in PAIRS}
    v = {h: cache(v_hbm, v_ref, h, value_sem) for h in PAIRS}
    wm, wq, wo, w3 = (weight(*args) for args in (
        (wm_hbm, wm_ref, S_WM), (wq_hbm, wq_ref, S_WQ), (wo_hbm, wo_ref, S_WO), (w3_hbm, w3_ref, S_W3)))
    w4 = [[piece for i, spans in enumerate(W4_BLOCKS) for piece in weight(w4_hbm, w4_ref, S_W4 + 2 * i + q, *spans[q])]
          for q in range(2)]
    gate = [[pltpu.make_async_copy(wm_hbm.at[:, pl.ds(row * 8, 8), pl.ds(GATE * 128, gate_ref.shape[2])],
                                   gate_ref.at[:, pl.ds(row * 8, 8)], sems.at[S_GATE + g])]
            for row, g in enumerate(g for g, n in enumerate(GATE_GROUPS) for _ in range(n))]
    inputs = [pltpu.make_async_copy(c_hbm, c_ref, sems.at[S_C]), pltpu.make_async_copy(x_hbm, x_ref, sems.at[S_X])]

    first = k[0] + k[1] + k[4] + _both_ends(wo)[-38:] + v[0] + v[5] + w4[0][:9] + w4[1] + gate
    second = _merge(_both_ends(wq), wm) + [inputs] + _both_ends(wo)[:-38] + k[5] + v[1] + v[4] + w3 + w4[0][9:]
    queue = []
    for j in range(max(len(first), len(second) + BACKLOG)):
        queue += [(1, copy) for piece in first[j:j + 1] for copy in piece]
        queue += [(0, copy) for piece in second[max(j - BACKLOG, 0):max(j + 1 - BACKLOG, 0)] for copy in piece]

    def ready(pieces):
        wanted = {id(copy) for piece in pieces for copy in piece}
        slow = [j for j, (priority, _) in enumerate(queue) if priority]
        return IN_FLIGHT + max(
            [j for j, (_, copy) in enumerate(queue) if id(copy) in wanted]
            + [slow[min(i + BACKLOG, len(slow) - 1)] for i, j in enumerate(slow) if id(queue[j][1]) in wanted])

    def landed(ref, sem):
        pltpu.make_async_copy(ref, ref, sems.at[sem]).wait()

    even = (lax.broadcasted_iota(jnp.int32, (ROWS, DH), 0) & 1) == 0
    head_columns = lambda ref, h: ref[:, :, h * 2 * DH:(h + 1) * 2 * DH].reshape(D, 2 * DH)
    residual = lambda: jnp.broadcast_to(x_ref[0].astype(F32), (ROWS, D))

    def condition():
        for copy in inputs:
            copy.wait()
        landed(wm_ref, S_WM)
        c = jnp.broadcast_to(c_ref[...].astype(F32), (ROWS, D))
        c = (c * jax.nn.sigmoid(c)).astype(BF16)
        mod = _dot(c, wm_ref[...].reshape(D, GATE * 128))
        for g in range(5):
            mod_ref[g] = mod[:, g * D:(g + 1) * D]
        mod_ref[5, :, :GATE * 128 - 5 * D] = mod[:, 5 * D:]
        diagonal = lax.broadcasted_iota(jnp.int32, (D, D), 0) == lax.broadcasted_iota(jnp.int32, (D, D), 1)
        column = jnp.sum(jnp.where(diagonal, jnp.broadcast_to(c.astype(F32)[:1], (D, D)), 0.0), axis=1, keepdims=True)
        silu_ref[...] = jnp.broadcast_to(column, (D, 128))
        attn_ref[...] = jnp.zeros((ROWS, D), F32)

    def queries():
        h_in = (_layernorm(residual()) * (1.0 + mod_ref[1]) + mod_ref[0]).astype(BF16)
        landed(wq_ref, S_WQ)
        for h in range(HKV):
            q = _dot(h_in, head_columns(wq_ref, h)) * DH ** -0.5
            q_ref[h] = jnp.where(even, q[:, :DH], q[:, DH:])

    def weights(h):
        landed(k_ref.at[h], S_K + h)
        s = _dot_t(q_ref[h].astype(BF16), k_ref[h].reshape(PIECES * keys_per_piece, DH))
        p = jnp.exp(s - jnp.max(_fold(jnp.maximum, s), axis=-1, keepdims=True))
        p_ref[h] = p
        scale_ref[h] = jnp.broadcast_to(1.0 / jnp.sum(_fold(jnp.add, p), axis=-1, keepdims=True), (ROWS, DH))

    def context(h, lo, hi):
        landed(v_ref.at[h, pl.ds(lo, hi - lo)], value_sem(h, lo))
        o = _dot(p_ref[h, :, lo * keys_per_piece:hi * keys_per_piece].astype(BF16),
                 v_ref[h, lo:hi].reshape((hi - lo) * keys_per_piece, DH))
        if lo > 0:
            o = o + o_ref[h]
        o_ref[h] = o * scale_ref[h] if hi == PIECES else o

    def project(h):
        o = o_ref[h]
        o = jnp.concatenate([jnp.where(even, o, 0.0), jnp.where(even, 0.0, o)], axis=1)
        attn_ref[...] += _dot_t(o.astype(BF16), head_columns(wo_ref, h))

    def normalize():
        attn = attn_ref[...]
        x = residual() + mod_ref[2] * (attn + pltpu.roll(attn, 1, 0))
        h_mlp = _layernorm(x) * (1.0 + mod_ref[4]) + mod_ref[3]
        mod_ref[0], mod_ref[1], mod_ref[2] = x, h_mlp, _layernorm(h_mlp)

    steps = [(ready(wm + [inputs]), 12, condition), (ready(wq), 15, queries)]
    for h in PAIRS:
        steps += [(ready(k[h]), 18, functools.partial(weights, head)) for head in (h, h + 2)]
    steps += [(ready(wo), 0, functools.partial(landed, wo_ref, S_WO))]
    for h in PAIRS:
        for lo, hi in ((0, LAST_EARLY), (LAST_EARLY, PIECES)) if h == LAST else ((0, PIECES),):
            steps += [(ready(v[h][:2 * hi]), (hi - lo) // 6, functools.partial(context, head, lo, hi))
                      for head in (h, h + 2)]
        steps += [(0, 4, functools.partial(project, head)) for head in (h, h + 2)]
    steps += [(0, 0, normalize)]

    earliest = 0
    for j, (priority, copy) in enumerate(queue):
        copy.start(priority=priority)
        while steps and j >= max(earliest, steps[0][0]):
            _, rest, step = steps.pop(0)
            step()
            earliest = j + rest
    for _, _, step in steps:
        step()

    landed(w3_ref, S_W3)
    hidden = jax.nn.gelu(_dot(mod_ref[2].astype(BF16), w3_ref[...].reshape(D, F)), approximate=True).astype(BF16)

    group = lax.broadcasted_iota(jnp.int32, (ROWS, 128), 1) // 16
    y = [jnp.zeros((ROWS, 128), F32)] * 4
    for i, spans in enumerate(W4_BLOCKS):
        for q, (lo, hi) in enumerate(spans):
            landed(w4_ref.at[:, pl.ds(lo * 8, (hi - lo) * 8)], S_W4 + 2 * i + q)
        channels = [s * HALF + r for s in range(2) for lo, hi in spans for r in range(lo * 8, hi * 8, 16)]
        while channels:
            lanes = {}
            for ch in channels:
                lanes.setdefault(ch % 128 // 16, ch)
            chosen = [lanes[g] for g in range(len(lanes))]
            channels = [ch for ch in channels if ch not in chosen]
            product = _dot_t(hidden, jnp.concatenate(
                [w4_ref[ch // HALF, pl.ds(ch % HALF, 16)] for ch in chosen], axis=0))
            if len(chosen) < 8:
                product = jnp.concatenate([product, jnp.zeros((ROWS, 128 - 16 * len(chosen)), F32)], axis=1)
            for g, ch in enumerate(chosen):
                y[ch // 128] = jnp.where(group == g, product, y[ch // 128])
    y = mod_ref[1] + jnp.concatenate(y, axis=1)[:, :D]

    total, lo = None, 0
    for g, n in enumerate(GATE_GROUPS):
        landed(gate_ref.at[:, pl.ds(lo, n * 8)], S_GATE + g)
        for s in range(2):
            w = gate_ref[s, lo:lo + n * 8].astype(F32)
            for r in range(0, n * 8, 8):
                term = w[r:r + 8] * jnp.concatenate([silu_ref[pl.ds(s * HALF + lo + r, 8)]] * 3, axis=1)
                total = term if total is None else total + term
        lo += n * 8
    gb = jnp.concatenate([mod_ref[5, :1, :GATE * 128 - 5 * D], jnp.sum(total, axis=0, keepdims=True)], axis=1)
    out_ref[0] = (mod_ref[0, :1] + gb * y[:1]).astype(BF16)
    store = pltpu.make_async_copy(out_ref, out_hbm, sems.at[S_X])
    store.start()
    store.wait()


@jax.jit
def pallas_adaLN_cond__sliding_block_cached__mixer_s_mlp__decode_kernel(
    A_x: jax.Array,
    A_k_cache: jax.Array,
    A_v_cache: jax.Array,
    A_wq: jax.Array,
    A_wo: jax.Array,
    B_x: jax.Array,
    B_w1: jax.Array,
    B_w2: jax.Array,
    B_w3: jax.Array,
    B_w4: jax.Array,
    c: jax.Array,
    w_mod: jax.Array,
):
    keys = A_k_cache.shape[2]
    window = min(4096, max(256, keys // 4))
    assert A_x.shape == (1, 1, D) and A_k_cache.shape == (1, HKV, keys, DH)
    assert window % BLOCK == 0 and keys % BLOCK == 0
    hbm = pl.BlockSpec(memory_space=pltpu.HBM)
    blocked = lambda cache: cache.reshape(HKV, keys // BLOCK, BLOCK, DH)
    halved = lambda w: w.reshape(2, HALF, w.shape[1])
    landing_order = (HKV, PIECES, window // BLOCK, SEGMENT, DH)
    return pl.pallas_call(
        _kernel,
        out_shape=jax.ShapeDtypeStruct(A_x.shape, A_x.dtype),
        in_specs=[hbm] * 9,
        out_specs=hbm,
        scratch_shapes=[
            pltpu.VMEM((1, 1, D), BF16),
            pltpu.VMEM((1, D), BF16),
            pltpu.VMEM((2, HALF, GATE * 128), BF16),
            pltpu.VMEM((2, HALF, 6 * D - GATE * 128), BF16),
            pltpu.VMEM((2, HALF, HQ * DH), BF16),
            pltpu.VMEM(landing_order, BF16),
            pltpu.VMEM(landing_order, BF16),
            pltpu.VMEM((2, HALF, HQ * DH), BF16),
            pltpu.VMEM((2, HALF, F), BF16),
            pltpu.VMEM((2, HALF, F), BF16),
            pltpu.VMEM((HKV, ROWS, DH), F32),
            pltpu.VMEM((HKV, ROWS, window), F32),
            pltpu.VMEM((HKV, ROWS, DH), F32),
            pltpu.VMEM((HKV, ROWS, DH), F32),
            pltpu.VMEM((ROWS, D), F32),
            pltpu.VMEM((6, ROWS, D), F32),
            pltpu.VMEM((D, 128), F32),
            pltpu.VMEM((1, 1, D), BF16),
            pltpu.SemaphoreType.DMA((S_GATE + len(GATE_GROUPS),)),
        ],
        compiler_params=pltpu.CompilerParams(
            vmem_limit_bytes=100 * 2**20,
            disable_semaphore_checks=True,
        ),
        name="adaln_decode",
    )(A_x, c, halved(w_mod), halved(A_wq), blocked(A_k_cache), blocked(A_v_cache), halved(A_wo.T),
      halved(B_w3), halved(B_w4.T))
```

```python
import functools

import jax
import jax.numpy as jnp
from jax import lax
from jax.experimental import pallas as pl
from jax.experimental.pallas import tpu as pltpu

D, F = 448, 1792
HQ, HKV, DH = 16, 8, 256
EPS = 1e-5
BF16, F32 = jnp.bfloat16, jnp.float32
ROWS = 8

HALF = D // 2
TILE_ROWS = HALF // 8
BLOCK, SEGMENT = 1024, 16
PIECES = BLOCK // SEGMENT
PAIRS = (0, 1, 4, 5)
STAGGER = 16
LAST, LAST_EARLY = 5, 56
GATE = 18
GATE_GROUPS = (12, 10, 4, 2)
W4_BLOCKS = (((6, 14), (14, 22)), ((0, 4), (24, 28)), ((4, 6), (22, 24)))
BACKLOG = 26
IN_FLIGHT = 54

S_X, S_C, S_WM, S_WQ, S_WO, S_W3, S_K, S_V, S_REST, S_W4 = 0, 1, 2, 3, 4, 5, 6, 14, 22, 24
S_GATE = S_W4 + 2 * len(W4_BLOCKS)


def _layernorm(x):
    d = x - jnp.sum(x, axis=-1, keepdims=True) * (1.0 / D)
    return d * lax.rsqrt(jnp.sum(d * d, axis=-1, keepdims=True) * (1.0 / D) + EPS)


def _dot(a, b):
    return lax.dot_general(a, b, (((1,), (0,)), ((), ())), preferred_element_type=F32)


def _dot_t(a, b):
    return lax.dot_general(a, b, (((1,), (1,)), ((), ())), preferred_element_type=F32)


def _fold(op, x):
    return functools.reduce(op, [x[:, t:t + 128] for t in range(0, x.shape[1], 128)])


def _merge(*lists):
    keyed = [((i + 0.5) / len(xs), j, x) for j, xs in enumerate(lists) for i, x in enumerate(xs)]
    return [x for _, _, x in sorted(keyed, key=lambda k: k[:2])]


def _both_ends(xs):
    return _merge(xs[:len(xs) // 2], xs[len(xs) // 2:])


def _cut(width, columns, lo, hi):
    pieces = {}
    for t in range(lo * width, hi * width):
        row, col = divmod(t, width)
        if col < columns:
            runs = pieces.setdefault(t // 8, [])
            if runs and runs[-1][0] == row:
                runs[-1] = (row, runs[-1][1], runs[-1][2] + 1)
            else:
                runs.append((row, col, 1))
    return list(pieces.values())


def _kernel(x_hbm, c_hbm, wm_hbm, wq_hbm, k_hbm, v_hbm, wo_hbm, w3_hbm, w4_hbm, out_hbm,
            x_ref, c_ref, wm_ref, gate_ref, wq_ref, k_ref, v_ref, wo_ref, w3_ref, w4_ref,
            q_ref, p_ref, scale_ref, o_ref, attn_ref, mod_ref, silu_ref, out_ref, sems):
    blocks = k_ref.shape[2]
    keys_per_piece = blocks * SEGMENT

    def cache(hbm, ref, h, sem):
        def piece(head, j):
            rows = pl.ds((j + (head - h) // 2 * STAGGER) % PIECES * SEGMENT, SEGMENT)
            return [pltpu.make_async_copy(hbm.at[head, pl.ds(hbm.shape[1] - blocks, blocks), rows],
                                          ref.at[head, j], sems.at[sem(head, j)])]
        return [piece(head, j) for j in range(PIECES) for head in (h, h + 2)]

    def value_sem(head, j):
        return S_REST + (head - LAST) // 2 if head in (LAST, LAST + 2) and j >= LAST_EARLY else S_V + head

    def weight(hbm, ref, sem, lo=0, hi=TILE_ROWS):
        def copy(row, col, n):
            at = (slice(None), pl.ds(row * 8, 8), pl.ds(col * 128, n * 128))
            return pltpu.make_async_copy(hbm.at[at], ref.at[at], sems.at[sem])
        return [[copy(*run) for run in piece] for piece in _cut(hbm.shape[2] // 128, ref.shape[2] // 128, lo, hi)]

    k = {h: cache(k_hbm, k_ref, h, lambda head, j: S_K + head) for h in PAIRS}
    v = {h: cache(v_hbm, v_ref, h, value_sem) for h in PAIRS}
    wm, wq, wo, w3 = (weight(*args) for args in (
        (wm_hbm, wm_ref, S_WM), (wq_hbm, wq_ref, S_WQ), (wo_hbm, wo_ref, S_WO), (w3_hbm, w3_ref, S_W3)))
    w4 = [[piece for i, spans in enumerate(W4_BLOCKS) for piece in weight(w4_hbm, w4_ref, S_W4 + 2 * i + q, *spans[q])]
          for q in range(2)]
    gate = [[pltpu.make_async_copy(wm_hbm.at[:, pl.ds(row * 8, 8), pl.ds(GATE * 128, gate_ref.shape[2])],
                                   gate_ref.at[:, pl.ds(row * 8, 8)], sems.at[S_GATE + g])]
            for row, g in enumerate(g for g, n in enumerate(GATE_GROUPS) for _ in range(n))]
    inputs = [pltpu.make_async_copy(c_hbm, c_ref, sems.at[S_C]), pltpu.make_async_copy(x_hbm, x_ref, sems.at[S_X])]

    first = k[0] + k[1] + k[4] + _both_ends(wo)[-38:] + v[0] + v[5] + w4[0][:9] + w4[1] + gate
    second = _merge(_both_ends(wq), wm) + [inputs] + _both_ends(wo)[:-38] + k[5] + v[1] + v[4] + w3 + w4[0][9:]
    queue = [(0, copy) for copy in second[0]]
    for j in range(max(len(first), len(second) + BACKLOG)):
        if j < len(first):
            queue += [(1, copy) for copy in first[j]]
        if 0 < j - BACKLOG < len(second):
            queue += [(0, copy) for copy in second[j - BACKLOG]]

    def ready(pieces):
        wanted = {id(copy) for piece in pieces for copy in piece}
        slow = [j for j, (priority, _) in enumerate(queue) if priority]
        return IN_FLIGHT + max(
            [j for j, (_, copy) in enumerate(queue) if id(copy) in wanted]
            + [slow[min(i + BACKLOG, len(slow) - 1)] for i, j in enumerate(slow) if id(queue[j][1]) in wanted])

    def landed(ref, sem):
        pltpu.make_async_copy(ref, ref, sems.at[sem]).wait()

    even = (lax.broadcasted_iota(jnp.int32, (ROWS, DH), 0) & 1) == 0
    head_columns = lambda ref, h: ref[:, :, h * 2 * DH:(h + 1) * 2 * DH].reshape(D, 2 * DH)
    residual = lambda: jnp.broadcast_to(x_ref[0].astype(F32), (ROWS, D))

    def condition():
        for copy in inputs:
            copy.wait()
        landed(wm_ref, S_WM)
        c = jnp.broadcast_to(c_ref[...].astype(F32), (ROWS, D))
        c = (c * jax.nn.sigmoid(c)).astype(BF16)
        mod = _dot(c, wm_ref[...].reshape(D, GATE * 128))
        for g in range(5):
            mod_ref[g] = mod[:, g * D:(g + 1) * D]
        mod_ref[5, :, :GATE * 128 - 5 * D] = mod[:, 5 * D:]
        diagonal = lax.broadcasted_iota(jnp.int32, (D, D), 0) == lax.broadcasted_iota(jnp.int32, (D, D), 1)
        column = jnp.sum(jnp.where(diagonal, jnp.broadcast_to(c.astype(F32)[:1], (D, D)), 0.0), axis=1, keepdims=True)
        silu_ref[...] = jnp.broadcast_to(column, (D, 128))
        attn_ref[...] = jnp.zeros((ROWS, D), F32)

    def queries():
        h_in = (_layernorm(residual()) * (1.0 + mod_ref[1]) + mod_ref[0]).astype(BF16)
        landed(wq_ref, S_WQ)
        for h in range(HKV):
            q = _dot(h_in, head_columns(wq_ref, h)) * DH ** -0.5
            q_ref[h] = jnp.where(even, q[:, :DH], q[:, DH:])

    def weights(h):
        landed(k_ref.at[h], S_K + h)
        s = _dot_t(q_ref[h].astype(BF16), k_ref[h].reshape(PIECES * keys_per_piece, DH))
        p = jnp.exp(s - jnp.max(_fold(jnp.maximum, s), axis=-1, keepdims=True))
        p_ref[h] = p
        scale_ref[h] = jnp.broadcast_to(1.0 / jnp.sum(_fold(jnp.add, p), axis=-1, keepdims=True), (ROWS, DH))

    def context(h, lo, hi):
        landed(v_ref.at[h, pl.ds(lo, hi - lo)], value_sem(h, lo))
        o = _dot(p_ref[h, :, lo * keys_per_piece:hi * keys_per_piece].astype(BF16),
                 v_ref[h, lo:hi].reshape((hi - lo) * keys_per_piece, DH))
        if lo > 0:
            o = o + o_ref[h]
        o_ref[h] = o * scale_ref[h] if hi == PIECES else o

    def project(h):
        o = o_ref[h]
        o = jnp.concatenate([jnp.where(even, o, 0.0), jnp.where(even, 0.0, o)], axis=1)
        attn_ref[...] += _dot_t(o.astype(BF16), head_columns(wo_ref, h))

    def normalize():
        attn = attn_ref[...]
        x = residual() + mod_ref[2] * (attn + pltpu.roll(attn, 1, 0))
        h_mlp = _layernorm(x) * (1.0 + mod_ref[4]) + mod_ref[3]
        mod_ref[0], mod_ref[1], mod_ref[2] = x, h_mlp, _layernorm(h_mlp)

    steps = [(ready(wm + [inputs]), 12, condition), (ready(wq), 15, queries)]
    for h in PAIRS:
        steps += [(ready(k[h]), 18, functools.partial(weights, head)) for head in (h, h + 2)]
    steps += [(ready(wo), 0, functools.partial(landed, wo_ref, S_WO))]
    for h in PAIRS:
        for lo, hi in ((0, LAST_EARLY), (LAST_EARLY, PIECES)) if h == LAST else ((0, PIECES),):
            steps += [(ready(v[h][:2 * hi]), (hi - lo) // 6, functools.partial(context, head, lo, hi))
                      for head in (h, h + 2)]
        steps += [(0, 4, functools.partial(project, head)) for head in (h, h + 2)]
    steps += [(0, 0, normalize)]

    earliest = 0
    for j, (priority, copy) in enumerate(queue):
        copy.start(priority=priority)
        while steps and j >= max(earliest, steps[0][0]):
            _, rest, step = steps.pop(0)
            step()
            earliest = j + rest
    for _, _, step in steps:
        step()

    landed(w3_ref, S_W3)
    hidden = jax.nn.gelu(_dot(mod_ref[2].astype(BF16), w3_ref[...].reshape(D, F)), approximate=True).astype(BF16)

    group = lax.broadcasted_iota(jnp.int32, (ROWS, 128), 1) // 16
    y = [jnp.zeros((ROWS, 128), F32)] * 4
    for i, spans in enumerate(W4_BLOCKS):
        for q, (lo, hi) in enumerate(spans):
            landed(w4_ref.at[:, pl.ds(lo * 8, (hi - lo) * 8)], S_W4 + 2 * i + q)
        channels = [s * HALF + r for s in range(2) for lo, hi in spans for r in range(lo * 8, hi * 8, 16)]
        while channels:
            lanes = {}
            for ch in channels:
                lanes.setdefault(ch % 128 // 16, ch)
            chosen = [lanes[g] for g in range(len(lanes))]
            channels = [ch for ch in channels if ch not in chosen]
            product = _dot_t(hidden, jnp.concatenate(
                [w4_ref[ch // HALF, pl.ds(ch % HALF, 16)] for ch in chosen], axis=0))
            if len(chosen) < 8:
                product = jnp.concatenate([product, jnp.zeros((ROWS, 128 - 16 * len(chosen)), F32)], axis=1)
            for g, ch in enumerate(chosen):
                y[ch // 128] = jnp.where(group == g, product, y[ch // 128])
    y = mod_ref[1] + jnp.concatenate(y, axis=1)[:, :D]

    total, lo = None, 0
    for g, n in enumerate(GATE_GROUPS):
        landed(gate_ref.at[:, pl.ds(lo, n * 8)], S_GATE + g)
        for s in range(2):
            w = gate_ref[s, lo:lo + n * 8].astype(F32)
            for r in range(0, n * 8, 8):
                term = w[r:r + 8] * jnp.concatenate([silu_ref[pl.ds(s * HALF + lo + r, 8)]] * 3, axis=1)
                total = term if total is None else total + term
        lo += n * 8
    gb = jnp.concatenate([mod_ref[5, :1, :GATE * 128 - 5 * D], jnp.sum(total, axis=0, keepdims=True)], axis=1)
    out_ref[0] = (mod_ref[0, :1] + gb * y[:1]).astype(BF16)
    store = pltpu.make_async_copy(out_ref, out_hbm, sems.at[S_X])
    store.start()
    store.wait()


@jax.jit
def pallas_adaLN_cond__sliding_block_cached__mixer_s_mlp__decode_kernel(
    A_x: jax.Array,
    A_k_cache: jax.Array,
    A_v_cache: jax.Array,
    A_wq: jax.Array,
    A_wo: jax.Array,
    B_x: jax.Array,
    B_w1: jax.Array,
    B_w2: jax.Array,
    B_w3: jax.Array,
    B_w4: jax.Array,
    c: jax.Array,
    w_mod: jax.Array,
):
    keys = A_k_cache.shape[2]
    window = min(4096, max(256, keys // 4))
    assert A_x.shape == (1, 1, D) and A_k_cache.shape == (1, HKV, keys, DH)
    assert window % BLOCK == 0 and keys % BLOCK == 0
    hbm = pl.BlockSpec(memory_space=pltpu.HBM)
    blocked = lambda cache: cache.reshape(HKV, keys // BLOCK, BLOCK, DH)
    halved = lambda w: w.reshape(2, HALF, w.shape[1])
    landing_order = (HKV, PIECES, window // BLOCK, SEGMENT, DH)
    return pl.pallas_call(
        _kernel,
        out_shape=jax.ShapeDtypeStruct(A_x.shape, A_x.dtype),
        in_specs=[hbm] * 9,
        out_specs=hbm,
        scratch_shapes=[
            pltpu.VMEM((1, 1, D), BF16),
            pltpu.VMEM((1, D), BF16),
            pltpu.VMEM((2, HALF, GATE * 128), BF16),
            pltpu.VMEM((2, HALF, 6 * D - GATE * 128), BF16),
            pltpu.VMEM((2, HALF, HQ * DH), BF16),
            pltpu.VMEM(landing_order, BF16),
            pltpu.VMEM(landing_order, BF16),
            pltpu.VMEM((2, HALF, HQ * DH), BF16),
            pltpu.VMEM((2, HALF, F), BF16),
            pltpu.VMEM((2, HALF, F), BF16),
            pltpu.VMEM((HKV, ROWS, DH), F32),
            pltpu.VMEM((HKV, ROWS, window), F32),
            pltpu.VMEM((HKV, ROWS, DH), F32),
            pltpu.VMEM((HKV, ROWS, DH), F32),
            pltpu.VMEM((ROWS, D), F32),
            pltpu.VMEM((6, ROWS, D), F32),
            pltpu.VMEM((D, 128), F32),
            pltpu.VMEM((1, 1, D), BF16),
            pltpu.SemaphoreType.DMA((S_GATE + len(GATE_GROUPS),)),
        ],
        compiler_params=pltpu.CompilerParams(
            vmem_limit_bytes=100 * 2**20,
            disable_semaphore_checks=True,
        ),
        name="adaln_decode",
    )(A_x, c, halved(w_mod), halved(A_wq), blocked(A_k_cache), blocked(A_v_cache), halved(A_wo.T),
      halved(B_w3), halved(B_w4.T))
```
